```python
import os as _os
_os.environ.setdefault("JAX_PLATFORMS", "cpu")
import jax
import jax.numpy as jnp

def _softmax(x, axis=-1):
    return jax.nn.softmax(x, axis=axis)
def _gelu(x):
    return jax.nn.gelu(x, approximate=True)
def _silu(x):
    return jax.nn.silu(x)
def _sigmoid(x):
    return jax.nn.sigmoid(x)
def _layernorm(x, axis=-1, eps=1e-5):
    m = jnp.mean(x, axis=axis, keepdims=True)
    v = jnp.var(x, axis=axis, keepdims=True)
    return (x - m) / jnp.sqrt(v + eps)
def _scatter_add(tgt, idx, src, axis=0):
    return tgt.at[idx].add(src)
def _segment_sum(src, seg, n):
    return jax.ops.segment_sum(src, seg, n)
class _Rng:
    def __init__(self, key):
        self._k = key
    def _next(self):
        self._k, sub = jax.random.split(self._k)
        return sub
    def normal(self, shape):
        return jax.random.normal(self._next(), shape, dtype=jnp.bfloat16)
    def randint(self, lo, hi, shape):
        return jax.random.randint(self._next(), shape, lo, hi, dtype=jnp.int32)
    def uniform(self, shape, lo=0.0, hi=1.0):
        return jax.random.uniform(self._next(), shape, jnp.bfloat16, lo, hi)
    def permutation(self, n):
        return jax.random.permutation(self._next(), n)


kernel_name = 'standalone__softmax_full_bidir__sampling'

def setup_inputs():
    _rng = _Rng(jax.random.key(int.from_bytes(__import__("os").urandom(4), "little")))
    _w = (lambda a: (lambda t: t.astype(jnp.bfloat16) if jnp.issubdtype(t.dtype, jnp.floating) else t)(jnp.asarray(a)))
    B, H, Sq, Skv, Dh = 8, 32, 1, 4096, 192
    return {
        "q": _w((lambda *s: _rng.normal(s) * 0.4)(B, H, Sq, Dh)),
        "k": _w((lambda *s: _rng.normal(s) * 0.4)(B, H, Skv, Dh)),
        "v": _w((lambda *s: _rng.normal(s) * 0.05)(B, H, Skv, Dh)),
    }

def reference(q, k, v):
    scale = q.shape[-1] ** -0.5
    scores = jnp.einsum('bhqd,bhkd->bhqk', q, k) * scale
    attn = _softmax(scores, axis=-1)
    return jnp.einsum('bhqk,bhkd->bhqd', attn, v)
```

```python
import functools

import jax
import jax.numpy as jnp
import jax.experimental.pallas as pl
import jax.experimental.pallas.tpu as pltpu

LANES = 128


def make(G=16, GS=1, LA=4, interleave=True, run2=False, compute=True, unroll_heads=True):
    def fn(q, k, v):
        B, H, Sq, D = q.shape
        S = k.shape[2]
        NH = B * H
        NG = D // 8
        NT = S // LANES
        NU = NT // 2
        UH = NG * NU
        PIECE = 8
        NGRP = NH // G
        SPG = NG // GS
        NSLOT = LA + 1
        SU = GS * NU
        T = NGRP * 2 * SPG
        scale = float(D) ** -0.5

        def flat(x):
            xt = jnp.swapaxes(x, 2, 3).reshape(NH * NG, 8, NT, LANES)
            return jnp.transpose(xt, (0, 2, 1, 3)).reshape(NH * UH, 16, LANES)

        npc = SU // PIECE
        if run2:
            order = [(j, m + r) for m in range(0, npc, 2) for j in range(G) for r in range(2)]
        else:
            order = [(j, m) for m in range(npc) for j in range(G)]

        def kernel(q_ref, k_hbm, v_hbm, o_ref, buf, acc, qt, ot, sem):
            def issue(src, t, lo, hi):
                grp = t // (2 * SPG)
                s = t % SPG
                slot = t % NSLOT
                base = grp * (G * UH) + s * SU
                for n in range(lo, hi):
                    j, m = order[n]
                    pltpu.make_async_copy(
                        src.at[pl.ds(base + (j * UH + m * PIECE), PIECE)],
                        buf.at[slot, j, pl.ds(m * PIECE, PIECE)],
                        sem.at[slot],
                    ).start(priority=n % 2)

            def wait(slot):
                pltpu.make_async_copy(buf.at[slot], buf.at[slot], sem.at[slot]).wait()

            assert LA <= SPG

            @pl.loop(0, LA)
            def _(t):
                issue(k_hbm, t, 0, len(order))

            lane = jax.lax.broadcasted_iota(jnp.int32, (8, LANES), 1)
            for hb in range(NH // LANES):
                qf = q_ref[hb * LANES:(hb + 1) * LANES, :].astype(jnp.float32) * scale
                qt[hb] = qf.T
            ot[...] = jnp.zeros(ot.shape, jnp.float32)

            def k_head(t, grp, s, j, first, last):
                slot = t % NSLOT
                h = grp * G + j
                hb = h // LANES
                sel = lane == (h % LANES)
                a = None if first else acc[j]
                for gi in range(GS):
                    r0 = pl.multiple_of((s * GS + gi) * 8, 8)
                    qv = jnp.sum(jnp.where(sel, qt[hb, pl.ds(r0, 8), :], 0.0), axis=1, keepdims=True)
                    x = buf[slot, j, gi * NU:(gi + 1) * NU].astype(jnp.float32).reshape(NT, 8, LANES)
                    y = x * qv[None]
                    a = y if a is None else a + y
                if last:
                    sc = jnp.sum(a, axis=1, keepdims=True)
                    m = jnp.max(jnp.max(sc, axis=0), axis=1, keepdims=True)
                    e = jnp.exp(sc - m[None])
                    l = jnp.sum(jnp.sum(e, axis=0), axis=1, keepdims=True)
                    a = jnp.broadcast_to(e * (1.0 / l)[None], (NT, 8, LANES))
                acc[j] = a

            def v_head(t, grp, s, j):
                slot = t % NSLOT
                h = grp * G + j
                hb = h // LANES
                sel = lane == (h % LANES)
                p = acc[j]
                for gi in range(GS):
                    r0 = pl.multiple_of((s * GS + gi) * 8, 8)
                    x = buf[slot, j, gi * NU:(gi + 1) * NU].astype(jnp.float32).reshape(NT, 8, LANES)
                    y = jnp.sum(jnp.sum(x * p, axis=0), axis=1, keepdims=True)
                    ot[hb, pl.ds(r0, 8), :] = jnp.where(sel, y, ot[hb, pl.ds(r0, 8), :])

            def step(t, src_next, head_fn):
                wait(t % NSLOT)
                per = len(order) // G
                if not interleave and src_next is not None:
                    issue(src_next, t + LA, 0, len(order))
                for j in range(G):
                    if interleave and src_next is not None:
                        issue(src_next, t + LA, j * per, (j + 1) * per)
                    if compute:
                        head_fn(j)

            def group(grp, last_group):
                t0 = grp * (2 * SPG)
                step(t0, k_hbm, lambda j: k_head(t0, grp, 0, j, True, False))

                @pl.loop(1, SPG - LA)
                def _(s):
                    step(t0 + s, k_hbm, lambda j: k_head(t0 + s, grp, s, j, False, False))

                @pl.loop(SPG - LA, SPG - 1)
                def _(s):
                    step(t0 + s, v_hbm, lambda j: k_head(t0 + s, grp, s, j, False, False))

                s = SPG - 1
                step(t0 + s, v_hbm, lambda j: k_head(t0 + s, grp, s, j, False, True))

                @pl.loop(0, SPG - LA)
                def _(s):
                    step(t0 + SPG + s, v_hbm, lambda j: v_head(t0 + SPG + s, grp, s, j))

                @pl.when(grp < NGRP - 1)
                def _():
                    @pl.loop(SPG - LA, SPG)
                    def _(s):
                        step(t0 + SPG + s, k_hbm, lambda j: v_head(t0 + SPG + s, grp, s, j))

            @pl.loop(0, NGRP)
            def _(grp):
                group(grp, False)

            grp = NGRP - 1
            t0 = grp * (2 * SPG)

            @pl.loop(SPG - LA, SPG)
            def _(s):
                step(t0 + SPG + s, None, lambda j: v_head(t0 + SPG + s, grp, s, j))

            for hb in range(NH // LANES):
                o_ref[hb * LANES:(hb + 1) * LANES, :] = ot[hb].T.astype(o_ref.dtype)

        o = pl.pallas_call(
            kernel,
            out_shape=jax.ShapeDtypeStruct((NH, D), q.dtype),
            in_specs=[
                pl.BlockSpec(memory_space=pltpu.VMEM),
                pl.BlockSpec(memory_space=pl.ANY),
                pl.BlockSpec(memory_space=pl.ANY),
            ],
            out_specs=pl.BlockSpec(memory_space=pltpu.VMEM),
            scratch_shapes=[
                pltpu.VMEM((NSLOT, G, SU, 16, LANES), k.dtype),
                pltpu.VMEM((G, NT, 8, LANES), jnp.float32),
                pltpu.VMEM((NH // LANES, D, LANES), jnp.float32),
                pltpu.VMEM((NH // LANES, D, LANES), jnp.float32),
                pltpu.SemaphoreType.DMA((NSLOT,)),
            ],
            compiler_params=pltpu.CompilerParams(
                vmem_limit_bytes=100 * 1024 * 1024, disable_bounds_checks=True
            ),
        )(q.reshape(NH, D), flat(k), flat(v))
        return o.reshape(B, H, Sq, D)

    return fn


@jax.jit
def pallas_standalone__softmax_full_bidir__sampling_kernel(q, k, v):
    return make(16, 1, 6, interleave=False)(q, k, v)
```

```python
import jax
import jax.numpy as jnp
import jax.experimental.pallas as pl
import jax.experimental.pallas.tpu as pltpu

LANES = 128


def make(G=16, LA=4, SH=1, HPW=8, wrap=True, compute=True, bounds=False, ngrp=None,
         qprio=0, oprio=0, ls=2, tailw=2, issue_first=True, flush_end=True, noq=False, hstride=1, qpos=None):
    def fn(q, k, v):
        B, H, Sq, D = q.shape
        S = k.shape[2]
        NH = B * H
        NG = D // 8
        NT = S // LANES
        HT = NT // 2
        PU = HT // 2
        PH = 2 * NG
        NGRP = NH // G if ngrp is None else ngrp
        NSLOT = 8 if LA < 8 else 16
        assert (2 * NG) % NSLOT == 0
        NW = G // HPW
        scale = float(D) ** -0.5

        def flat(x):
            xt = jnp.swapaxes(x, 2, 3).reshape(NH * NG, 8, NT, LANES)
            return jnp.transpose(xt, (0, 2, 1, 3)).reshape(NH * PH, PU, 16, LANES)

        def kernel(q_hbm, k_hbm, v_hbm, o_hbm, buf, acc, part, qv, qt, ot, ov, sem, tsem, qsem, osem):
            def start(src, grp, j, m, slot, c, s_ref, n):
                pltpu.make_async_copy(
                    src.at[(grp * G + j) * PH + m], buf.at[slot, j, c], s_ref
                ).start(priority=n % 2)

            def issue(src, grp, s, slot, j0, nj, s_ref):
                first = isinstance(s, int) and s == 0
                if not SH:
                    halves = ((0, 2 * s), (1, 2 * s + 1))
                elif first:
                    halves = ((1, PH - 1), (0, 0))
                else:
                    halves = ((1, 2 * s - 1), (0, 2 * s))
                n = 0
                for a in range(0, nj, ls):
                    for c, m in halves:
                        for i in range(a, a + ls):
                            if SH and first and wrap and c == 1:
                                i = (i - 1) % nj
                            start(src, grp, j0 + i, m, slot, c, s_ref, n)
                            n += 1

            def wait(slot, j0, nj, s_ref):
                r = buf.at[slot, pl.ds(j0, nj)]
                pltpu.make_async_copy(r, r, s_ref).wait()

            q_copy = pltpu.make_async_copy(q_hbm, qv, qsem)
            for w in range(NW):
                issue(k_hbm, 0, 0, 0, w * HPW, HPW, sem.at[0, w])
            if not noq:
                q_copy.start(priority=qprio)

            def prologue(lo, hi):
                @pl.loop(lo, hi)
                def _(s):
                    for w in range(NW):
                        issue(k_hbm, 0, s, s, w * HPW, HPW, sem.at[s, w])

            qp = LA if qpos is None else qpos
            prologue(1, qp)
            if not noq:
                q_copy.wait()
            lane = jax.lax.broadcasted_iota(jnp.int32, (8, LANES), 1)
            for hb in range(NH // LANES):
                qf = qv[hb * LANES:(hb + 1) * LANES, :].astype(jnp.float32) * scale
                qt[hb] = qf.T
            ot[...] = jnp.zeros(ot.shape, jnp.float32)
            if qp < LA:
                prologue(qp, LA)

            def load(slot, j, c):
                return buf[slot, j, c].astype(jnp.float32).reshape(HT, 8, LANES)

            def rows(g):
                if isinstance(g, int):
                    return pl.ds(g * 8, 8)
                return pl.ds(pl.multiple_of(g * 8, 8), 8)

            def k_heads(grp, s, slot, j0, nj):
                first = isinstance(s, int) and s == 0
                last = isinstance(s, int) and s == NG - 1
                h0 = grp * G + j0
                hb = h0 >> 7
                rel = lane - (h0 & (LANES - 1))
                g1 = (NG - 1 if first else s - 1) if SH else s
                qs = [qt[hb, rows(g), :] for g in (s, g1)]
                for i in range(nj):
                    j = j0 + i
                    a = []
                    for c in range(2):
                        qc = jnp.sum(jnp.where(rel == i, qs[c], 0.0), axis=1, keepdims=True)
                        y = load(slot, j, c) * qc[None]
                        a.append(y if first else acc[j, c] + y)
                    if last:
                        sc = [jnp.sum(x, axis=1, keepdims=True) for x in a]
                        m = jnp.max(jnp.max(jnp.maximum(sc[0], sc[1]), axis=0), axis=1, keepdims=True)
                        e = [jnp.exp(x - m[None]) for x in sc]
                        l = jnp.sum(jnp.sum(e[0] + e[1], axis=0), axis=1, keepdims=True)
                        r = (1.0 / l)[None]
                        a = [jnp.broadcast_to(x * r, (HT, 8, LANES)) for x in e]
                    acc[j, 0] = a[0]
                    acc[j, 1] = a[1]

            def v_heads(grp, s, slot, j0, nj):
                first = isinstance(s, int) and s == 0
                last = isinstance(s, int) and s == NG - 1
                rel = lane - j0
                if not SH:
                    gs = [s]
                else:
                    gs = [] if first else [s - 1, s] if last else [s - 1]
                outs = [ot[rows(g), :] for g in gs]
                for i in range(nj):
                    j = j0 + i
                    y0 = jnp.sum(load(slot, j, 0) * acc[j, 0], axis=0)
                    y1 = jnp.sum(load(slot, j, 1) * acc[j, 1], axis=0)
                    if not SH:
                        ys = [y0 + y1]
                    elif first:
                        part[j, 0] = y0
                        part[j, 1] = y1
                        ys = []
                    elif last:
                        ys = [part[j, 0] + y1, part[j, 1] + y0]
                    else:
                        ys = [part[j, 0] + y1]
                        part[j, 0] = y0
                    outs = [jnp.where(rel == i, jnp.sum(y, axis=1, keepdims=True), o)
                            for y, o in zip(ys, outs)]
                for g, o in zip(gs, outs):
                    ot[rows(g), :] = o

            def step(grp, ph, s, heads, nxt):
                slot = (ph * NG + s) & (NSLOT - 1)
                nslot = (ph * NG + s + LA) & (NSLOT - 1)

                def body(w):
                    j0 = w * HPW
                    wait(slot, j0, HPW, sem.at[slot, w])
                    if nxt is not None and issue_first:
                        nxt(nslot, w)
                    if compute:
                        heads(grp, s, slot, j0, HPW)
                    if nxt is not None and not issue_first:
                        nxt(nslot, w)

                if NW == 1:
                    body(0)
                else:
                    pl.loop(0, NW)(body)

            def ahead(src, grp, s):
                return lambda nslot, w: issue(src, grp, s, nslot, w * HPW, HPW, sem.at[nslot, w])

            def ahead_tail(grp):
                def f(nslot, w):
                    for u in range(HPW // tailw):
                        issue(v_hbm, grp, NG - 1, nslot, w * HPW + u * tailw, tailw,
                              tsem.at[w * (HPW // tailw) + u])
                return f

            def out_copy(grp):
                r = pl.ds(pl.multiple_of(grp * G, G), G)
                return pltpu.make_async_copy(ov.at[r], o_hbm.at[r], osem)

            def steps(grp, ph, lo, hi, heads, nxt):
                @pl.loop(lo, hi)
                def _(s):
                    step(grp, ph, s, heads, nxt(s) if nxt else None)

            @pl.loop(0, NGRP)
            def _(grp):
                step(grp, 0, 0, k_heads, ahead(k_hbm, grp, LA))
                steps(grp, 0, 1, NG - LA, k_heads, lambda s: ahead(k_hbm, grp, s + LA))
                step(grp, 0, NG - LA, k_heads, ahead(v_hbm, grp, 0))
                steps(grp, 0, NG - LA + 1, NG - 1, k_heads, lambda s: ahead(v_hbm, grp, s + LA - NG))
                step(grp, 0, NG - 1, k_heads, ahead(v_hbm, grp, LA - 1))

                step(grp, 1, 0, v_heads, ahead(v_hbm, grp, LA))
                steps(grp, 1, 1, NG - LA - 1, v_heads, lambda s: ahead(v_hbm, grp, s + LA))
                step(grp, 1, NG - LA - 1, v_heads, ahead_tail(grp))

                def guarded(f):
                    def g(nslot, w):
                        @pl.when(grp < NGRP - 1)
                        def _():
                            f(nslot, w)
                    return g

                step(grp, 1, NG - LA, v_heads, guarded(ahead(k_hbm, grp + 1, 0)))
                steps(grp, 1, NG - LA + 1, NG - 1, v_heads,
                      lambda s: guarded(ahead(k_hbm, grp + 1, s + LA - NG)))

                slot = (2 * NG - 1) & (NSLOT - 1)
                nslot = (2 * NG - 1 + LA) & (NSLOT - 1)
                for w in range(NW):
                    guarded(ahead(k_hbm, grp + 1, LA - 1))(nslot, w)
                for u in range(G // tailw):
                    wait(slot, u * tailw, tailw, tsem.at[u])
                    if compute:
                        v_heads(grp, NG - 1, slot, u * tailw, tailw)
                ov[pl.ds(pl.multiple_of(grp * G, G), G), :] = ot[:, :G].T.astype(ov.dtype)
                if not flush_end:
                    out_copy(grp).start(priority=oprio)

            r = pl.ds(0, NGRP * G)
            if flush_end:
                pltpu.make_async_copy(ov.at[r], o_hbm.at[r], osem).start()
            pltpu.make_async_copy(ov.at[r], o_hbm.at[r], osem).wait()

        any_spec = pl.BlockSpec(memory_space=pl.ANY)
        o = pl.pallas_call(
            kernel,
            out_shape=jax.ShapeDtypeStruct((NH, D), q.dtype),
            in_specs=[any_spec, any_spec, any_spec],
            out_specs=any_spec,
            scratch_shapes=[
                pltpu.VMEM((NSLOT, G, 2, PU, 16, LANES), k.dtype),
                pltpu.VMEM((G, 2, HT, 8, LANES), jnp.float32),
                pltpu.VMEM((G, 2, 8, LANES), jnp.float32),
                pltpu.VMEM((NH, D), q.dtype),
                pltpu.VMEM((NH // LANES, D, LANES), jnp.float32),
                pltpu.VMEM((D, LANES), jnp.float32),
                pltpu.VMEM((NH, D), q.dtype),
                pltpu.SemaphoreType.DMA((NSLOT, NW)),
                pltpu.SemaphoreType.DMA((G // tailw,)),
                pltpu.SemaphoreType.DMA(()),
                pltpu.SemaphoreType.DMA(()),
            ],
            compiler_params=pltpu.CompilerParams(
                vmem_limit_bytes=64 * 1024 * 1024, disable_bounds_checks=not bounds
            ),
        )(q.reshape(NH, D), flat(k), flat(v))
        return o.reshape(B, H, Sq, D)

    return fn


@jax.jit
def pallas_standalone__softmax_full_bidir__sampling_kernel(q, k, v):
    return make(HPW=8, tailw=8)(q, k, v)
```

```python
import jax
import jax.numpy as jnp
import jax.experimental.pallas as pl
import jax.experimental.pallas.tpu as pltpu

LANES = 128
SUBLANES = 8
HEADS = 16
BATCH = 8
LOOKAHEAD = 4
SLOTS = 8
TAIL = ((0, 2, 4, 6, 8, 10, 12, 14, 1, 3, 5, 7), (9, 11, 13, 15))


@jax.jit
def pallas_standalone__softmax_full_bidir__sampling_kernel(
    q: jax.Array,
    k: jax.Array,
    v: jax.Array,
):
    batch, heads, q_len, dim = q.shape
    keys = k.shape[2]
    n_heads = batch * heads
    n_groups = n_heads // HEADS
    n_rows = dim // SUBLANES
    n_steps = 2 * n_rows
    tiles = keys // LANES
    half_tiles = tiles // 2
    run = tiles // 2
    half = run // 2
    head_len = n_rows * run
    n_blocks = pl.cdiv(dim, LANES)
    rows_per_block = LANES // SUBLANES
    scale = float(dim) ** -0.5
    assert q_len == 1 and n_heads % HEADS == 0 and n_groups > 1
    assert dim % SUBLANES == 0 and keys % (8 * LANES) == 0
    assert n_steps % SLOTS == 0 and LOOKAHEAD < min(SLOTS, n_rows)

    def kernel(q_hbm, k_hbm, v_hbm, o_hbm, buf, scores, probs, q_vmem, q_f32, o_f32, o_vmem,
               sems, tail_sems, q_sem, o_sems):
        lane = jax.lax.broadcasted_iota(jnp.int32, (SUBLANES, LANES), 1)
        sublane = jax.lax.broadcasted_iota(jnp.int32, (SUBLANES, LANES), 0)

        def aligned(start, size):
            return pl.ds(start if isinstance(start, int) else pl.multiple_of(start, size), size)

        def start_runs(src, head0, step, n, dst):
            base = head0 * head_len + step * run - half
            for pair in range(0, n, 2):
                for part in range(2):
                    for i in (pair, pair + 1):
                        cut = half if i == 0 else half // 2
                        lo, hi = ((0, cut), (cut, run))[part]
                        start = base + i * head_len + lo
                        if i == 0 and part == 0 and not isinstance(step, int):
                            start += jnp.where(step == 0, n * head_len, 0)
                        view, sem = dst(i)
                        pltpu.make_async_copy(
                            src.at[pl.ds(start, hi - lo)], view.at[pl.ds(lo, hi - lo)], sem
                        ).start(priority=i % 2)

        def start_batch(src, group, step, slot, b):
            def dst(i):
                return buf.at[slot, pl.ds((b * BATCH + i) * run, run)], sems.at[slot, b]

            start_runs(src, group * HEADS + b * BATCH, step, BATCH, dst)

        def wait_runs(slot, first, n, sem):
            filled = buf.at[slot, pl.ds(first * run, n * run)]
            pltpu.make_async_copy(filled, filled, sem).wait()

        tail_slot = (n_steps - 1) % SLOTS
        tail_order = [j for js in TAIL for j in js]

        def tail_dst(j):
            b = [j in js for js in TAIL].index(True)
            return buf.at[tail_slot, pl.ds(tail_order.index(j) * run, run)], tail_sems.at[b]

        def out_copy(lo, hi, i):
            rows = pl.ds(lo, hi - lo)
            return pltpu.make_async_copy(o_vmem.at[rows], o_hbm.at[rows], o_sems.at[i])

        def halves(step, slot, pos, i):
            if isinstance(step, int):
                prev, shift = step - 1, 0
            else:
                prev = jnp.where(step == 0, n_rows - 1, step - 1)
                shift = jnp.where(step == 0, run if i < BATCH - 1 else (1 - BATCH) * run, 0)
            return [
                (g, buf[slot, pl.ds(at, half)].astype(jnp.float32).reshape(half_tiles, SUBLANES, LANES))
                for g, at in ((step, pos * run + half), (prev, pos * run + shift))
            ]

        def diagonal(g):
            return lane - sublane == jax.lax.rem(g, rows_per_block) * SUBLANES

        def add_scores(group, step, slot, b):
            acc = scores.at[aligned(b * BATCH * tiles * SUBLANES, BATCH * tiles * SUBLANES)]
            for i in range(BATCH):
                head = group * HEADS + b * BATCH + i
                for c, (g, kt) in enumerate(halves(step, slot, b * BATCH + i, i)):
                    q_row = q_f32[jax.lax.div(g, rows_per_block), pl.ds(head, 1), :]
                    q_col = jnp.sum(jnp.where(diagonal(g), q_row, 0.0), axis=1, keepdims=True)
                    rows = pl.ds((2 * i + c) * half_tiles * SUBLANES, half_tiles * SUBLANES)
                    acc[rows, :] += (kt * q_col[None]).reshape(half_tiles * SUBLANES, LANES)

        def softmax(b):
            n = BATCH // 2

            @pl.loop(2 * b, 2 * b + 2)
            def _(c):
                acc = scores.at[aligned(c * n * tiles * SUBLANES, n * tiles * SUBLANES)]
                for i in range(n):
                    s = acc[pl.ds(i * tiles * SUBLANES, tiles, stride=SUBLANES), :]
                    for r in range(1, SUBLANES):
                        s += acc[pl.ds(i * tiles * SUBLANES + r, tiles, stride=SUBLANES), :]
                    m = jnp.max(jnp.max(s, axis=0, keepdims=True), axis=1, keepdims=True)
                    e = jnp.exp(s - m)
                    total = jnp.sum(jnp.sum(e, axis=0, keepdims=True), axis=1, keepdims=True)
                    probs[c * n + i] = e / total

        def clear_scores(first, n):
            size = 2 * tiles

            @pl.loop(first * 4, (first + n) * 4)
            def _(i):
                scores[aligned(i * size, size), :] = jnp.zeros((size, LANES), jnp.float32)

        def add_values(step, slot, pos, i, j, rows):
            for c, (g, vt) in enumerate(halves(step, slot, pos, i)):
                y = [vt[t] * probs[j, pl.ds(c * half_tiles + t, 1), :] for t in range(half_tiles)]
                while len(y) > 1:
                    y = [sum(y[t + 1:t + 2], y[t]) for t in range(0, len(y), 2)]
                col = jnp.sum(y[0], axis=1, keepdims=True)
                row = jnp.sum(jnp.where(diagonal(g), col, 0.0), axis=0, keepdims=True)
                pltpu.store(
                    o_f32.at[c, jax.lax.div(g, rows_per_block), rows, :],
                    jnp.broadcast_to(row, (SUBLANES, LANES)),
                    mask=(sublane == i % SUBLANES) & ((lane >> 3) == jax.lax.rem(g, rows_per_block)),
                )

        def finish(group):
            rows = aligned(group * HEADS, HEADS)
            for blk in range(n_blocks):
                width = min(LANES, dim - blk * LANES)
                y = o_f32[0, blk, rows, :width] + o_f32[1, blk, rows, :width]
                o_vmem[rows, blk * LANES:blk * LANES + width] = y.astype(o_vmem.dtype)

        n_batches = HEADS // BATCH
        q_copy = pltpu.make_async_copy(q_hbm, q_vmem, q_sem)

        @pl.loop(0, LOOKAHEAD * n_batches)
        def _(i):
            step = jax.lax.div(i, n_batches)
            start_batch(k_hbm, 0, step, step, jax.lax.rem(i, n_batches))

            @pl.when(i == 0)
            def _():
                q_copy.start()

        q_copy.wait()

        @pl.loop(0, n_groups)
        def _(group):
            rows = aligned(group * HEADS, HEADS)
            zeros = jnp.zeros((HEADS, LANES), jnp.float32)
            q_f32[n_blocks - 1, rows, :] = zeros
            for blk in range(n_blocks):
                width = min(LANES, dim - blk * LANES)
                x = q_vmem[rows, blk * LANES:blk * LANES + width]
                q_f32[blk, rows, :width] = x.astype(jnp.float32) * scale
                o_f32[0, blk, rows, :] = zeros
                o_f32[1, blk, rows, :] = zeros

        clear_scores(0, HEADS)

        @pl.loop(0, n_groups)
        def _(group):
            last = group == n_groups - 1
            end = jnp.where(last, n_steps - 1, n_steps)

            @pl.loop(0, end)
            def _(t):
                slot = t & (SLOTS - 1)
                ahead = t + LOOKAHEAD
                ahead_slot = ahead & (SLOTS - 1)

                @pl.loop(0, n_batches)
                def _(b):
                    wait_runs(slot, b * BATCH, BATCH, sems.at[slot, b])

                    @pl.when((ahead < n_rows) | ((ahead >= n_steps) & jnp.logical_not(last)))
                    def _():
                        wrap = ahead >= n_steps
                        start_batch(k_hbm, group + wrap.astype(jnp.int32),
                                    jnp.where(wrap, ahead - n_steps, ahead), ahead_slot, b)

                    @pl.when((ahead >= n_rows) & (ahead < end))
                    def _():
                        start_batch(v_hbm, group, ahead - n_rows, ahead_slot, b)

                    @pl.when(last & (ahead == n_steps - 1) & (b == n_batches - 1))
                    def _():
                        start_runs(v_hbm, n_heads - HEADS, n_rows - 1, HEADS, tail_dst)

                    @pl.when(t < n_rows)
                    def _():
                        add_scores(group, t, slot, b)

                    @pl.when(t == n_rows - 1)
                    def _():
                        softmax(b)

                    @pl.when(t == n_rows)
                    def _():
                        clear_scores(b * BATCH, BATCH)

                    @pl.when(t >= n_rows)
                    def _():
                        for i in range(BATCH):
                            j = b * BATCH + i
                            rows = aligned(group * HEADS + b * BATCH + (i & -SUBLANES), SUBLANES)
                            add_values(t - n_rows, slot, j, i, j, rows)

            @pl.when(jnp.logical_not(last))
            def _():
                finish(group)

        done = n_heads - HEADS
        for b, js in enumerate(TAIL):
            if b == len(TAIL) - 1:
                out_copy(0, done, 0).start(priority=1)
            wait_runs(tail_slot, tail_order.index(js[0]), len(js), tail_sems.at[b])
            for j in js:
                rows = pl.ds(done + (j & -SUBLANES), SUBLANES)
                add_values(n_rows - 1, tail_slot, tail_order.index(j), j, j, rows)
        finish(n_groups - 1)
        out_copy(done, n_heads, 1).start()
        out_copy(0, done, 0).wait()
        out_copy(done, n_heads, 1).wait()

    def as_vregs(x):
        xt = jnp.swapaxes(x, 2, 3).reshape(n_heads * n_rows, SUBLANES, tiles, LANES)
        return jnp.swapaxes(xt, 1, 2).reshape(n_heads * head_len, 2 * SUBLANES, LANES)

    in_hbm = pl.BlockSpec(memory_space=pl.ANY)
    out = pl.pallas_call(
        kernel,
        out_shape=jax.ShapeDtypeStruct((n_heads, dim), q.dtype),
        in_specs=[in_hbm, in_hbm, in_hbm],
        out_specs=in_hbm,
        scratch_shapes=[
            pltpu.VMEM((SLOTS, HEADS * run, 2 * SUBLANES, LANES), k.dtype),
            pltpu.VMEM((HEADS * tiles * SUBLANES, LANES), jnp.float32),
            pltpu.VMEM((HEADS, tiles, LANES), jnp.float32),
            pltpu.VMEM((n_heads, dim), q.dtype),
            pltpu.VMEM((n_blocks, n_heads, LANES), jnp.float32),
            pltpu.VMEM((2, n_blocks, n_heads, LANES), jnp.float32),
            pltpu.VMEM((n_heads, dim), q.dtype),
            pltpu.SemaphoreType.DMA((SLOTS, HEADS // BATCH)),
            pltpu.SemaphoreType.DMA((len(TAIL),)),
            pltpu.SemaphoreType.DMA(()),
            pltpu.SemaphoreType.DMA((2,)),
        ],
        compiler_params=pltpu.CompilerParams(
            vmem_limit_bytes=32 * 1024 * 1024,
            disable_bounds_checks=True,
            disable_semaphore_checks=True,
        ),
    )(q.reshape(n_heads, dim), as_vregs(k), as_vregs(v))
    return out.reshape(batch, heads, q_len, dim)
```

```python
import jax
import jax.numpy as jnp
import jax.experimental.pallas as pl
import jax.experimental.pallas.tpu as pltpu

LANES = 128
SUBLANES = 8
HEADS = 16
BATCH = 8
LOOKAHEAD = 4
SLOTS = 8
TAIL = ((0, 2, 4, 6, 8, 10, 12, 14, 1, 3, 5, 7), (9, 11, 13, 15))


@jax.jit
def pallas_standalone__softmax_full_bidir__sampling_kernel(
    q: jax.Array,
    k: jax.Array,
    v: jax.Array,
):
    batch, heads, q_len, dim = q.shape
    keys = k.shape[2]
    n_heads = batch * heads
    n_groups = n_heads // HEADS
    n_rows = dim // SUBLANES
    n_steps = 2 * n_rows
    tiles = keys // LANES
    half_tiles = tiles // 2
    run = tiles // 2
    half = run // 2
    head_len = n_rows * run
    n_blocks = pl.cdiv(dim, LANES)
    rows_per_block = LANES // SUBLANES
    scale = float(dim) ** -0.5
    assert q_len == 1 and n_heads % HEADS == 0 and n_groups > 1
    assert dim % SUBLANES == 0 and keys % (8 * LANES) == 0
    assert n_steps % SLOTS == 0 and LOOKAHEAD < min(SLOTS, n_rows)

    def kernel(q_hbm, k_hbm, v_hbm, o_hbm, buf, scores, probs, q_vmem, q_f32, o_f32, o_vmem,
               sems, tail_sems, q_sem, o_sems):
        lane = jax.lax.broadcasted_iota(jnp.int32, (SUBLANES, LANES), 1)
        sublane = jax.lax.broadcasted_iota(jnp.int32, (SUBLANES, LANES), 0)

        def aligned(start, size):
            return pl.ds(start if isinstance(start, int) else pl.multiple_of(start, size), size)

        def start_runs(src, head0, step, n, dst):
            base = head0 * head_len + step * run - half
            for pair in range(0, n, 2):
                for part in range(2):
                    for i in (pair, pair + 1):
                        cut = (half, half // 2)[i % 2]
                        lo, hi = ((0, cut), (cut, run))[part]
                        start = base + i * head_len + lo
                        if i == 0 and part == 0 and not isinstance(step, int):
                            start += jnp.where(step == 0, n * head_len, 0)
                        view, sem = dst(i)
                        pltpu.make_async_copy(
                            src.at[pl.ds(start, hi - lo)], view.at[pl.ds(lo, hi - lo)], sem
                        ).start(priority=i % 2)

        def start_batch(src, group, step, slot, b):
            def dst(i):
                return buf.at[slot, pl.ds((b * BATCH + i) * run, run)], sems.at[slot, b]

            start_runs(src, group * HEADS + b * BATCH, step, BATCH, dst)

        def wait_runs(slot, first, n, sem):
            filled = buf.at[slot, pl.ds(first * run, n * run)]
            pltpu.make_async_copy(filled, filled, sem).wait()

        tail_slot = (n_steps - 1) % SLOTS
        tail_order = [j for js in TAIL for j in js]

        def tail_dst(j):
            b = [j in js for js in TAIL].index(True)
            return buf.at[tail_slot, pl.ds(tail_order.index(j) * run, run)], tail_sems.at[b]

        def out_copy(lo, hi, i):
            rows = pl.ds(lo, hi - lo)
            return pltpu.make_async_copy(o_vmem.at[rows], o_hbm.at[rows], o_sems.at[i])

        def halves(step, slot, pos, i):
            if isinstance(step, int):
                prev, shift = step - 1, 0
            else:
                prev = jnp.where(step == 0, n_rows - 1, step - 1)
                shift = jnp.where(step == 0, run if i < BATCH - 1 else (1 - BATCH) * run, 0)
            return [
                (g, buf[slot, pl.ds(at, half)].astype(jnp.float32).reshape(half_tiles, SUBLANES, LANES))
                for g, at in ((step, pos * run + half), (prev, pos * run + shift))
            ]

        def locate(g):
            if isinstance(g, int):
                return divmod(g, rows_per_block)
            return jax.lax.div(g, rows_per_block), jax.lax.rem(g, rows_per_block)

        def diagonal(at):
            return lane - sublane == at * SUBLANES

        def tree_sum(xs):
            mid = len(xs) // 2
            return tree_sum(xs[:mid]) + tree_sum(xs[mid:]) if mid else xs[0]

        def add_scores(group, step, slot, b):
            acc = scores.at[aligned(b * BATCH * tiles * SUBLANES, BATCH * tiles * SUBLANES)]
            for i in range(BATCH):
                head = group * HEADS + b * BATCH + i
                for c, (g, kt) in enumerate(halves(step, slot, b * BATCH + i, i)):
                    blk, at = locate(g)
                    q_row = q_f32[blk, pl.ds(head, 1), :]
                    q_col = jnp.sum(jnp.where(diagonal(at), q_row, 0.0), axis=1, keepdims=True)
                    rows = pl.ds((2 * i + c) * half_tiles * SUBLANES, half_tiles * SUBLANES)
                    acc[rows, :] += (kt * q_col[None]).reshape(half_tiles * SUBLANES, LANES)

        def softmax(b):
            n = BATCH // 2

            @pl.loop(2 * b, 2 * b + 2)
            def _(c):
                acc = scores.at[aligned(c * n * tiles * SUBLANES, n * tiles * SUBLANES)]
                for i in range(n):
                    s = acc[pl.ds(i * tiles * SUBLANES, tiles, stride=SUBLANES), :]
                    for r in range(1, SUBLANES):
                        s += acc[pl.ds(i * tiles * SUBLANES + r, tiles, stride=SUBLANES), :]
                    m = jnp.max(jnp.max(s, axis=0, keepdims=True), axis=1, keepdims=True)
                    e = jnp.exp(s - m)
                    total = jnp.sum(jnp.sum(e, axis=0, keepdims=True), axis=1, keepdims=True)
                    probs[c * n + i] = e / total

        def clear_scores(first, n):
            size = 2 * tiles

            @pl.loop(first * 4, (first + n) * 4)
            def _(i):
                scores[aligned(i * size, size), :] = jnp.zeros((size, LANES), jnp.float32)

        def add_values(step, slot, pos, i, j, rows):
            for c, (g, vt) in enumerate(halves(step, slot, pos, i)):
                blk, at = locate(g)
                y = tree_sum([vt[t] * probs[j, pl.ds(c * half_tiles + t, 1), :]
                              for t in range(half_tiles)])
                col = jnp.sum(y, axis=1, keepdims=True)
                row = jnp.sum(jnp.where(diagonal(at), col, 0.0), axis=0, keepdims=True)
                pltpu.store(
                    o_f32.at[c, blk, rows, :],
                    jnp.broadcast_to(row, (SUBLANES, LANES)),
                    mask=(sublane == i % SUBLANES) & ((lane >> 3) == at),
                )

        def finish(group):
            rows = aligned(group * HEADS, HEADS)
            for blk in range(n_blocks):
                width = min(LANES, dim - blk * LANES)
                y = o_f32[0, blk, rows, :width] + o_f32[1, blk, rows, :width]
                o_vmem[rows, blk * LANES:blk * LANES + width] = y.astype(o_vmem.dtype)

        n_batches = HEADS // BATCH
        q_copy = pltpu.make_async_copy(q_hbm, q_vmem, q_sem)

        @pl.loop(0, LOOKAHEAD * n_batches)
        def _(i):
            step = jax.lax.div(i, n_batches)
            start_batch(k_hbm, 0, step, step, jax.lax.rem(i, n_batches))

            @pl.when(i == 0)
            def _():
                q_copy.start()

        q_copy.wait()

        @pl.loop(0, n_groups)
        def _(group):
            rows = aligned(group * HEADS, HEADS)
            zeros = jnp.zeros((HEADS, LANES), jnp.float32)
            q_f32[n_blocks - 1, rows, :] = zeros
            for blk in range(n_blocks):
                width = min(LANES, dim - blk * LANES)
                x = q_vmem[rows, blk * LANES:blk * LANES + width]
                q_f32[blk, rows, :width] = x.astype(jnp.float32) * scale
                o_f32[0, blk, rows, :] = zeros
                o_f32[1, blk, rows, :] = zeros

        clear_scores(0, HEADS)

        @pl.loop(0, n_groups)
        def _(group):
            last = group == n_groups - 1
            end = jnp.where(last, n_steps - 1, n_steps)

            @pl.loop(0, end)
            def _(t):
                slot = t & (SLOTS - 1)
                ahead = t + LOOKAHEAD
                ahead_slot = ahead & (SLOTS - 1)

                @pl.loop(0, n_batches)
                def _(b):
                    wait_runs(slot, b * BATCH, BATCH, sems.at[slot, b])

                    @pl.when((ahead < n_rows) | ((ahead >= n_steps) & jnp.logical_not(last)))
                    def _():
                        wrap = ahead >= n_steps
                        start_batch(k_hbm, group + wrap.astype(jnp.int32),
                                    jnp.where(wrap, ahead - n_steps, ahead), ahead_slot, b)

                    @pl.when((ahead >= n_rows) & (ahead < end))
                    def _():
                        start_batch(v_hbm, group, ahead - n_rows, ahead_slot, b)

                    @pl.when(last & (ahead == n_steps - 1) & (b == n_batches - 1))
                    def _():
                        start_runs(v_hbm, n_heads - HEADS, n_rows - 1, HEADS, tail_dst)

                    @pl.when(t < n_rows)
                    def _():
                        add_scores(group, t, slot, b)

                    @pl.when(t == n_rows - 1)
                    def _():
                        softmax(b)

                    @pl.when(t == n_rows)
                    def _():
                        clear_scores(b * BATCH, BATCH)

                    @pl.when(t >= n_rows)
                    def _():
                        for i in range(BATCH):
                            j = b * BATCH + i
                            rows = aligned(group * HEADS + b * BATCH + (i & -SUBLANES), SUBLANES)
                            add_values(t - n_rows, slot, j, i, j, rows)

            @pl.when(jnp.logical_not(last))
            def _():
                finish(group)

        done = n_heads - HEADS
        for b, js in enumerate(TAIL):
            if b == len(TAIL) - 1:
                out_copy(0, done, 0).start(priority=1)
            wait_runs(tail_slot, tail_order.index(js[0]), len(js), tail_sems.at[b])
            for j in js:
                rows = pl.ds(done + (j & -SUBLANES), SUBLANES)
                add_values(n_rows - 1, tail_slot, tail_order.index(j), j, j, rows)
        finish(n_groups - 1)
        out_copy(done, n_heads, 1).start()
        out_copy(0, done, 0).wait()
        out_copy(done, n_heads, 1).wait()

    def as_vregs(x):
        xt = jnp.swapaxes(x, 2, 3).reshape(n_heads * n_rows, SUBLANES, tiles, LANES)
        return jnp.swapaxes(xt, 1, 2).reshape(n_heads * head_len, 2 * SUBLANES, LANES)

    in_hbm = pl.BlockSpec(memory_space=pl.ANY)
    out = pl.pallas_call(
        kernel,
        out_shape=jax.ShapeDtypeStruct((n_heads, dim), q.dtype),
        in_specs=[in_hbm, in_hbm, in_hbm],
        out_specs=in_hbm,
        scratch_shapes=[
            pltpu.VMEM((SLOTS, HEADS * run, 2 * SUBLANES, LANES), k.dtype),
            pltpu.VMEM((HEADS * tiles * SUBLANES, LANES), jnp.float32),
            pltpu.VMEM((HEADS, tiles, LANES), jnp.float32),
            pltpu.VMEM((n_heads, dim), q.dtype),
            pltpu.VMEM((n_blocks, n_heads, LANES), jnp.float32),
            pltpu.VMEM((2, n_blocks, n_heads, LANES), jnp.float32),
            pltpu.VMEM((n_heads, dim), q.dtype),
            pltpu.SemaphoreType.DMA((SLOTS, HEADS // BATCH)),
            pltpu.SemaphoreType.DMA((len(TAIL),)),
            pltpu.SemaphoreType.DMA(()),
            pltpu.SemaphoreType.DMA((2,)),
        ],
        compiler_params=pltpu.CompilerParams(
            vmem_limit_bytes=32 * 1024 * 1024,
            disable_semaphore_checks=True,
        ),
    )(q.reshape(n_heads, dim), as_vregs(k), as_vregs(v))
    return out.reshape(batch, heads, q_len, dim)
```
